```python
import jax
import jax.numpy as jnp

def _softmax(x, axis=-1):
    return jax.nn.softmax(x, axis=axis)
def _gelu(x):
    return jax.nn.gelu(x, approximate=True)
def _silu(x):
    return jax.nn.silu(x)
def _sigmoid(x):
    return jax.nn.sigmoid(x)
def _layernorm(x, axis=-1, eps=1e-5):
    m = jnp.mean(x, axis=axis, keepdims=True)
    v = jnp.var(x, axis=axis, keepdims=True)
    return (x - m) / jnp.sqrt(v + eps)
def _scatter_add(tgt, idx, src, axis=0):
    return tgt.at[idx].add(src)
def _segment_sum(src, seg, n):
    return jax.ops.segment_sum(src, seg, n)
class _Rng:
    def __init__(self, key):
        self._k = key
    def _next(self):
        self._k, sub = jax.random.split(self._k)
        return sub
    def normal(self, shape):
        return jax.random.normal(self._next(), shape, dtype=jnp.bfloat16)
    def randint(self, lo, hi, shape):
        return jax.random.randint(self._next(), shape, lo, hi, dtype=jnp.int32)
    def uniform(self, shape, lo=0.0, hi=1.0):
        return jax.random.uniform(self._next(), shape, jnp.bfloat16, lo, hi)
    def permutation(self, n):
        return jax.random.permutation(self._next(), n)


kernel_name = 'sequential_preLN__compressed_kv_cla__moe_arch_mod__decode'

def setup_inputs():
    _rng = _Rng(jax.random.key(int.from_bytes(__import__("os").urandom(4), "little")))
    _w = (lambda a: (lambda t: t.astype(jnp.bfloat16) if jnp.issubdtype(t.dtype, jnp.floating) else t)(jnp.asarray(a)))
    def _A_setup():
        B, H, Sq, Sk, D, M = 1, 32, 1, 8192, 128, 512
        Dc = 4 * D
        return {
            "x": _w((lambda *s: _rng.normal(s) * 0.05)(B, Sq, M)),
            "c_kv": _w((lambda *s: _rng.normal(s) * 0.05)(B, Sk, Dc)),
            "w_q": _w((lambda *s: _rng.normal(s) * 0.05)(M, H, D) * (M ** -0.5)),
            "w_uk": _w((lambda *s: _rng.normal(s) * 0.05)(Dc, H, D) * (Dc ** -0.5)),
            "w_uv": _w((lambda *s: _rng.normal(s) * 0.05)(Dc, H, D) * (Dc ** -0.5)),
            "w_o": _w((lambda *s: _rng.normal(s) * 0.05)(H, D, M) * ((H * D) ** -0.5)),
        }
    _A_in = _A_setup()

    def _B_setup():
        B, S, D, F, C = 1, 1, 512, 1376, 1
        return {
            "x": _w((lambda *s: _rng.normal(s) * 0.05)(B, S, D)),
            "w_r": _w((lambda *s: _rng.normal(s) * 0.05)(D)),
            "w_gate": _w((lambda *s: _rng.normal(s) * 0.05)(D, F)),
            "w_up": _w((lambda *s: _rng.normal(s) * 0.05)(D, F)),
            "w_down": _w((lambda *s: _rng.normal(s) * 0.05)(F, D)),
        }
    _B_in = _B_setup()

    return {
        "A_x": _A_in["x"],
        "A_c_kv": _A_in["c_kv"],
        "A_w_q": _A_in["w_q"],
        "A_w_uk": _A_in["w_uk"],
        "A_w_uv": _A_in["w_uv"],
        "A_w_o": _A_in["w_o"],
        "B_x": _B_in["x"],
        "B_w_r": _B_in["w_r"],
        "B_w_gate": _B_in["w_gate"],
        "B_w_up": _B_in["w_up"],
        "B_w_down": _B_in["w_down"],
    }

def reference(A_x, A_c_kv, A_w_q, A_w_uk, A_w_uv, A_w_o, B_x, B_w_r, B_w_gate, B_w_up, B_w_down):
    def _A_ref(x, c_kv, w_q, w_uk, w_uv, w_o):
        B, Sq, M = x.shape[0], x.shape[1], x.shape[2]
        Sk = c_kv.shape[1]
        H, D = w_q.shape[1], w_q.shape[2]
        q = jnp.einsum("bqm,mhd->bhqd", x, w_q)
        k = jnp.einsum("bkc,chd->bhkd", c_kv, w_uk)
        v = jnp.einsum("bkc,chd->bhkd", c_kv, w_uv)
        scores = jnp.einsum("bhqd,bhkd->bhqk", q, k) * (D ** -0.5)
        off = Sk - Sq
        qi = jnp.arange(Sq)[:, None]
        kj = jnp.arange(Sk)[None, :]
        cmask = kj <= (qi + off)
        scores = jnp.where(cmask[None, None], scores, -1e9)
        p = _softmax(scores, axis=-1)
        ctx = jnp.einsum("bhqk,bhkd->bhqd", p, v)
        return jnp.einsum("bhqd,hdm->bqm", ctx, w_o)

    def _B_ref(x, w_r, w_gate, w_up, w_down):
        B, S, D = x.shape
        C = 1
        r = x @ w_r
        idx = jnp.argsort(-r, axis=-1)[:, :C]
        idx_e = jnp.repeat(idx.reshape(B, C, 1), D, axis=2)
        x_sel = jnp.take_along_axis(x, idx_e, axis=1)
        g = _silu(x_sel @ w_gate)
        u = x_sel @ w_up
        y = (g * u) @ w_down
        r_sel = _sigmoid(jnp.take_along_axis(r, idx, axis=1))
        y = y * r_sel.reshape(B, C, 1)
        b_off = (jnp.arange(B) * S).reshape(B, 1)
        flat_idx = (idx + b_off).reshape(B * C)
        zero = (x * 0.0).reshape(B * S, D)
        upd = _scatter_add(zero, flat_idx, y.reshape(B * C, D), axis=0)
        return x + upd.reshape(B, S, D)

    x = A_x
    h = x + _A_ref(_layernorm(x, axis=-1), A_c_kv, A_w_q, A_w_uk, A_w_uv, A_w_o)
    h2 = h + _B_ref(_layernorm(h, axis=-1), B_w_r, B_w_gate, B_w_up, B_w_down)
    return h2
```

```python
import functools
import jax
import jax.numpy as jnp
from jax import lax
import jax.experimental.pallas as pl
import jax.experimental.pallas.tpu as pltpu

BF = jnp.bfloat16
F32 = jnp.float32
NT = (((1,), (1,)), ((), ()))
EPS = 1e-5

DEFAULT = dict(tu=8, ckv_chunks=2, kb=512, ou=2, window=100, fchunk=256, dsplit=(1024,), skip=())


def _layernorm(v):
    m = jnp.mean(v, axis=-1, keepdims=True)
    d = v - m
    var = jnp.mean(d * d, axis=-1, keepdims=True)
    return d / jnp.sqrt(var + EPS)


def make(**kw):
    cfg = dict(DEFAULT); cfg.update(kw)
    H, D, M, SK, DC, F = 32, 128, 512, 8192, 512, 1376
    TU, NCK, KB, OU, WINDOW = cfg['tu'], cfg['ckv_chunks'], cfg['kb'], cfg['ou'], cfg['window']
    FCH = cfg['fchunk']
    dbounds = (0,) + tuple(cfg['dsplit']) + (F,)
    skip = cfg['skip']
    n_dma = 2 + 2 + NCK + 2 + 2 + len(dbounds) - 1

    def body(x_hbm, ckv_hbm, wq_hbm, wuk_hbm, wuv_hbm, wo_hbm, wr_hbm, wg_hbm, wu_hbm, wd_hbm, o_ref,
             x_v, wr_v, ckv_v, wq_v, wuk_v, wuv_v, wo_v, wg_v, wu_v, wd_v, e_ref, s_ref, ctx_ref, hm_ref, sems):
        copies = []
        def add(src, dst):
            copies.append(pltpu.make_async_copy(src, dst, sems.at[len(copies)]))
            return len(copies) - 1
        i_wq = add(wq_hbm, wq_v)
        i_x = add(x_hbm, x_v)
        i_wr = add(wr_hbm, wr_v)
        i_wuk = add(wuk_hbm, wuk_v)
        ck = SK // NCK
        i_ckv = [add(ckv_hbm.at[pl.ds(j * ck, ck)], ckv_v.at[pl.ds(j * ck, ck)]) for j in range(NCK)]
        i_wuv = add(wuv_hbm, wuv_v)
        i_wo = add(wo_hbm, wo_v)
        i_wg = add(wg_hbm, wg_v)
        i_wu = add(wu_hbm, wu_v)
        i_wd = [add(wd_hbm.at[pl.ds(a, b - a)], wd_v.at[pl.ds(a, b - a)]) for a, b in zip(dbounds[:-1], dbounds[1:])]
        started = [0]
        def start_upto(n):
            while started[0] < min(n, len(copies)):
                copies[started[0]].start()
                started[0] += 1
        def wait(i):
            start_upto(i + 1)
            copies[i].wait()
            start_upto(i + 1 + WINDOW)
        start_upto(2 + WINDOW)

        lane = lax.broadcasted_iota(jnp.int32, (H, 128), 1)
        row = lax.broadcasted_iota(jnp.int32, (H, 128), 0)
        diag = (lane % H) == row

        def w_tile(w_ref, t):
            return jnp.concatenate(
                [w_ref[pl.ds(pl.multiple_of((i * 128 + t) * H, H), H), :] for i in range(4)], axis=0)

        def head_proj(w_ref, y):
            e_ref[...] = y.T
            def step(tb, acc):
                lhs, rhs = [], []
                for u in range(TU):
                    t = tb * TU + u
                    coef = jnp.broadcast_to(e_ref[pl.ds(t, 1), :], (H, 128))
                    lhs.append(jnp.where(diag, coef, 0.0).astype(BF))
                    rhs.append(w_tile(w_ref, t))
                return acc + jnp.dot(jnp.concatenate(lhs, axis=1), jnp.concatenate(rhs, axis=0),
                                     preferred_element_type=F32)
            return lax.fori_loop(0, 128 // TU, step, jnp.zeros((H, D), F32))

        wait(i_x)
        x = x_v[0].astype(F32)
        xn = _layernorm(x)
        y = jnp.concatenate([jnp.broadcast_to(xn[:, i * 128:(i + 1) * 128], (H, 128)) for i in range(4)], axis=0)
        wait(i_wq)
        if 'q' in skip:
            q = y[:32].astype(BF)
        else:
            q = head_proj(wq_v, y).astype(BF)

        wait(i_wuk)
        def absorb(tb, carry):
            rhs = jnp.concatenate([w_tile(wuk_v, tb * TU + u) for u in range(TU)], axis=0)
            r = lax.dot_general(q, rhs, NT, preferred_element_type=F32)
            for u in range(TU):
                ru = jnp.where(diag, r[:, u * 128:(u + 1) * 128], 0.0)
                e_ref[pl.ds(tb * TU + u, 1), :] = jnp.sum(ru, axis=0, keepdims=True)
            return carry
        if 'qa' not in skip:
            lax.fori_loop(0, 128 // TU, absorb, 0)
        vt = e_ref[...].T * (D ** -0.5)
        qa = jnp.concatenate([vt[i * H:(i + 1) * H, :] for i in range(4)], axis=1).astype(BF)

        nb = ck // KB
        mx = jnp.full((H, 128), -jnp.inf, F32)
        for j in range(NCK):
            wait(i_ckv[j])
            def score(b, mx, j=j):
                blk = j * nb + b
                c = ckv_v[pl.ds(pl.multiple_of(blk * KB, KB), KB), :]
                s = lax.dot_general(qa, c, NT, preferred_element_type=F32)
                s_ref[blk] = s
                for u in range(KB // 128):
                    mx = jnp.maximum(mx, s[:, u * 128:(u + 1) * 128])
                return mx
            if 's' not in skip:
                mx = lax.fori_loop(0, nb, score, mx)
        m = jnp.max(mx, axis=1, keepdims=True)

        def pv(blk, carry):
            l, acc = carry
            p = jnp.exp(s_ref[blk] - m)
            for u in range(KB // 128):
                l = l + p[:, u * 128:(u + 1) * 128]
            c = ckv_v[pl.ds(pl.multiple_of(blk * KB, KB), KB), :]
            return l, acc + jnp.dot(p.astype(BF), c, preferred_element_type=F32)
        l, acc = jnp.zeros((H, 128), F32), jnp.zeros((H, DC), F32)
        if 'pv' not in skip:
            l, acc = lax.fori_loop(0, SK // KB, pv, (l, acc))
        cc = acc / jnp.sum(l, axis=1, keepdims=True)

        y = jnp.concatenate([cc[:, i * 128:(i + 1) * 128] for i in range(4)], axis=0)
        wait(i_wuv)
        if 'v' in skip:
            ctx_ref[...] = y[:32]
        else:
            ctx_ref[...] = head_proj(wuv_v, y)

        wait(i_wo)
        def oproj(hb, acc):
            lhs = jnp.concatenate(
                [jnp.broadcast_to(ctx_ref[pl.ds(hb * OU + u, 1), :], (16, D)) for u in range(OU)], axis=1)
            w = wo_v[pl.ds(pl.multiple_of(hb * (OU * D), OU * D), OU * D), :]
            return acc + jnp.dot(lhs.astype(BF), w, preferred_element_type=F32)
        attn = jnp.zeros((16, M), F32)
        if 'o' not in skip:
            attn = lax.fori_loop(0, H // OU, oproj, attn)
        h = x + attn[0:1]
        hn = _layernorm(h)

        wait(i_wr)
        wr = wr_v[...].astype(F32)
        r = sum(jnp.sum(hn[:, i * 128:(i + 1) * 128] * wr[i:i + 1], axis=1, keepdims=True) for i in range(4))
        hb16 = jnp.broadcast_to(hn, (16, M)).astype(BF)
        fb = list(range(0, F, FCH)) + [F]
        wait(i_wg)
        for a, b in zip(fb[:-1], fb[1:]):
            g = lax.dot_general(hb16, wg_v[a:b, :], NT, preferred_element_type=F32)
            hm_ref[:, a:b] = g * jax.nn.sigmoid(g)
        wait(i_wu)
        for a, b in zip(fb[:-1], fb[1:]):
            u = lax.dot_general(hb16, wu_v[a:b, :], NT, preferred_element_type=F32)
            hm_ref[:, a:b] = hm_ref[:, a:b] * u
        yv = jnp.zeros((16, M), F32)
        for j, (a, b) in enumerate(zip(dbounds[:-1], dbounds[1:])):
            wait(i_wd[j])
            yv = yv + jnp.dot(hm_ref[:, a:b].astype(BF), wd_v[a:b, :], preferred_element_type=F32)
        out = h + (hn + (hn * 0.0 + yv[0:1] * jax.nn.sigmoid(r)))
        o_ref[0] = out.astype(o_ref.dtype)

    @jax.jit
    def fn(A_x, A_c_kv, A_w_q, A_w_uk, A_w_uv, A_w_o, B_x, B_w_r, B_w_gate, B_w_up, B_w_down):
        del B_x
        return pl.pallas_call(
            body,
            out_shape=jax.ShapeDtypeStruct((1, 1, M), A_x.dtype),
            in_specs=[pl.BlockSpec(memory_space=pl.ANY)] * 10,
            scratch_shapes=[
                pltpu.VMEM((1, 1, M), BF), pltpu.VMEM((4, 128), BF),
                pltpu.VMEM((SK, DC), BF), pltpu.VMEM((M * H, D), BF), pltpu.VMEM((DC * H, D), BF),
                pltpu.VMEM((DC * H, D), BF), pltpu.VMEM((H * D, M), BF),
                pltpu.VMEM((F, M), BF), pltpu.VMEM((F, M), BF), pltpu.VMEM((F, M), BF),
                pltpu.VMEM((128, 128), F32), pltpu.VMEM((SK // KB, H, KB), F32), pltpu.VMEM((H, D), F32),
                pltpu.VMEM((16, F), F32),
                pltpu.SemaphoreType.DMA((n_dma,)),
            ],
            compiler_params=pltpu.CompilerParams(vmem_limit_bytes=64 * 2**20),
        )(A_x, A_c_kv.reshape(SK, DC), A_w_q.reshape(M * H, D), A_w_uk.reshape(DC * H, D),
          A_w_uv.reshape(DC * H, D), A_w_o.reshape(H * D, M), B_w_r.reshape(4, 128),
          B_w_gate.T, B_w_up.T, B_w_down)
    return fn


_kernel = make()


@jax.jit
def pallas_sequential_preLN__compressed_kv_cla__moe_arch_mod__decode_kernel(
    A_x, A_c_kv, A_w_q, A_w_uk, A_w_uv, A_w_o, B_x, B_w_r, B_w_gate, B_w_up, B_w_down):
    return _kernel(A_x, A_c_kv, A_w_q, A_w_uk, A_w_uv, A_w_o, B_x, B_w_r, B_w_gate, B_w_up, B_w_down)
```

```python
import jax
import jax.numpy as jnp
from jax import lax
import jax.experimental.pallas as pl
import jax.experimental.pallas.tpu as pltpu

BF = jnp.bfloat16
F32 = jnp.float32
NT = (((1,), (1,)), ((), ()))
EPS = 1e-5

H, D, M, SK, DC, F = 32, 128, 512, 8192, 512, 1376
LANES = 128
TILES = 8
KB = 512
OHEADS = 2
FCH = 256
NSEM = 3
DOWN_ROWS = (0, 640, 1024, 1264, 1344, F)
VPU_START = 1024
COL_TILES = -(-(F - VPU_START) // LANES)
COL_BASE = F - COL_TILES * LANES


def _layernorm(v):
    mean = jnp.mean(v, axis=-1, keepdims=True)
    d = v - mean
    var = jnp.mean(d * d, axis=-1, keepdims=True)
    return d / jnp.sqrt(var + EPS)


def _kernel(x_hbm, ckv_hbm, wq_hbm, wuk_hbm, wuv_hbm, wo_hbm, wr_hbm, wg_hbm, wu_hbm, wd_hbm,
            o_hbm,
            x_v, wr_v, ckv_v, wq_v, wuk_v, wuv_v, wo_v, wg_v, wu_v, wd_v,
            e_ref, s_ref, ctx_ref, hm_ref, y_ref, col_ref, o_v, sems):
    down_chunks = list(zip(DOWN_ROWS[:-1], DOWN_ROWS[1:]))
    groups = [
        [(wq_hbm, wq_v), (x_hbm, x_v), (wr_hbm, wr_v)],
        [(wuk_hbm, wuk_v)], [(ckv_hbm, ckv_v)], [(wuv_hbm, wuv_v)], [(wo_hbm, wo_v)],
        [(wg_hbm, wg_v)], [(wu_hbm, wu_v)],
    ] + [[(wd_hbm.at[pl.ds(a, b - a)], wd_v.at[pl.ds(a, b - a)])] for a, b in down_chunks]
    g_wq, g_wuk, g_ckv, g_wuv, g_wo, g_wg, g_wu, g_wd = range(8)
    copies = [[pltpu.make_async_copy(src, dst, sems.at[g % NSEM]) for src, dst in group]
              for g, group in enumerate(groups)]

    def start(g):
        if g < len(copies):
            for copy in copies[g]:
                copy.start()

    def wait(g):
        for copy in copies[g]:
            copy.wait()
        start(g + NSEM)

    for g in range(NSEM):
        start(g)

    lane = lax.broadcasted_iota(jnp.int32, (H, LANES), 1)
    row = lax.broadcasted_iota(jnp.int32, (H, LANES), 0)
    own_head = (lane % H) == row

    def w_tile(w_ref, t):
        return jnp.concatenate(
            [w_ref[pl.ds(pl.multiple_of((i * LANES + t) * H, H), H), :] for i in range(4)], axis=0)

    def head_proj(w_ref, coef):
        e_ref[...] = coef.T

        def step(tb, acc):
            lhs, rhs = [], []
            for u in range(TILES):
                t = tb * TILES + u
                a = jnp.broadcast_to(e_ref[pl.ds(t, 1), :], (H, LANES))
                lhs.append(jnp.where(own_head, a, 0.0).astype(BF))
                rhs.append(w_tile(w_ref, t))
            return acc + jnp.dot(jnp.concatenate(lhs, axis=1), jnp.concatenate(rhs, axis=0),
                                 preferred_element_type=F32)

        return lax.fori_loop(0, LANES // TILES, step, jnp.zeros((H, D), F32))

    wait(g_wq)
    x = x_v[0].astype(F32)
    xn = _layernorm(x)
    q = head_proj(wq_v, jnp.concatenate(
        [jnp.broadcast_to(xn[:, i * LANES:(i + 1) * LANES], (H, LANES)) for i in range(4)], axis=0))
    q = q.astype(BF)

    wait(g_wuk)

    def absorb(tb, carry):
        rhs = jnp.concatenate([w_tile(wuk_v, tb * TILES + u) for u in range(TILES)], axis=0)
        r = lax.dot_general(q, rhs, NT, preferred_element_type=F32)
        for u in range(TILES):
            own = jnp.where(own_head, r[:, u * LANES:(u + 1) * LANES], 0.0)
            e_ref[pl.ds(tb * TILES + u, 1), :] = jnp.sum(own, axis=0, keepdims=True)
        return carry

    lax.fori_loop(0, LANES // TILES, absorb, 0)
    qa = e_ref[...].T * (D ** -0.5)
    qa = jnp.concatenate([qa[i * H:(i + 1) * H, :] for i in range(4)], axis=1).astype(BF)

    wait(g_ckv)

    def score(blk, mx):
        c = ckv_v[pl.ds(pl.multiple_of(blk * KB, KB), KB), :]
        s = lax.dot_general(qa, c, NT, preferred_element_type=F32)
        s_ref[blk] = s
        for u in range(KB // LANES):
            mx = jnp.maximum(mx, s[:, u * LANES:(u + 1) * LANES])
        return mx

    mx = lax.fori_loop(0, SK // KB, score, jnp.full((H, LANES), -jnp.inf, F32))
    row_max = jnp.max(mx, axis=1, keepdims=True)

    def attend(blk, carry):
        den, acc = carry
        p = jnp.exp(s_ref[blk] - row_max)
        for u in range(KB // LANES):
            den = den + p[:, u * LANES:(u + 1) * LANES]
        c = ckv_v[pl.ds(pl.multiple_of(blk * KB, KB), KB), :]
        return den, acc + jnp.dot(p.astype(BF), c, preferred_element_type=F32)

    den, acc = lax.fori_loop(0, SK // KB, attend,
                             (jnp.zeros((H, LANES), F32), jnp.zeros((H, DC), F32)))
    cc = acc / jnp.sum(den, axis=1, keepdims=True)

    coef = jnp.concatenate([cc[:, i * LANES:(i + 1) * LANES] for i in range(4)], axis=0)
    wait(g_wuv)
    ctx_ref[...] = head_proj(wuv_v, coef)

    wait(g_wo)

    def out_proj(hb, acc):
        lhs = jnp.concatenate(
            [jnp.broadcast_to(ctx_ref[pl.ds(hb * OHEADS + u, 1), :], (16, D)) for u in range(OHEADS)],
            axis=1)
        w = wo_v[pl.ds(pl.multiple_of(hb * (OHEADS * D), OHEADS * D), OHEADS * D), :]
        return acc + jnp.dot(lhs.astype(BF), w, preferred_element_type=F32)

    attn = lax.fori_loop(0, H // OHEADS, out_proj, jnp.zeros((16, M), F32))
    h = x + attn[0:1]
    hn = _layernorm(h)

    wr = wr_v[...].astype(F32)
    r = sum(jnp.sum(hn[:, i * LANES:(i + 1) * LANES] * wr[i:i + 1], axis=1, keepdims=True)
            for i in range(4))
    route = jax.nn.sigmoid(r)
    hn16 = jnp.broadcast_to(hn, (16, M)).astype(BF)
    f_chunks = [(a, min(a + FCH, F)) for a in range(0, F, FCH)]
    wait(g_wg)
    for a, b in f_chunks:
        g = lax.dot_general(hn16, wg_v[a:b, :], NT, preferred_element_type=F32)
        hm_ref[:, a:b] = g * jax.nn.sigmoid(g) * route
    wait(g_wu)
    for a, b in f_chunks:
        u = lax.dot_general(hn16, wu_v[a:b, :], NT, preferred_element_type=F32)
        hm_ref[:, a:b] = hm_ref[:, a:b] * u
    for t in range(COL_TILES):
        lo = COL_BASE + t * LANES
        col_ref[t * LANES:(t + 1) * LANES, :] = jnp.broadcast_to(
            hm_ref[0:1, lo:lo + LANES], (LANES, LANES)).T

    y = jnp.broadcast_to(h + (hn + hn * 0.0), (16, M))
    y8 = None
    for j, (a, b) in enumerate(down_chunks):
        wait(g_wd + j)
        if a < VPU_START:
            y = y + jnp.dot(hm_ref[:, a:b].astype(BF), wd_v[a:b, :], preferred_element_type=F32)
            y_ref[...] = y
            continue
        if y8 is None:
            y8 = jnp.where(lax.broadcasted_iota(jnp.int32, (8, M), 0) == 0, y[0:8], 0.0)
        for r0 in range(a, b, 16):
            w = wd_v[r0:r0 + 16, :].astype(F32)
            unit = col_ref[r0 - COL_BASE:r0 - COL_BASE + 16, :]
            p = w * jnp.concatenate([unit] * (M // LANES), axis=1)
            y8 = y8 + (p[0:8] + p[8:16])
        if b < F:
            y_ref[0:8] = y8

    o_v[0] = jnp.sum(y8, axis=0, keepdims=True).astype(o_v.dtype)
    out = pltpu.make_async_copy(o_v, o_hbm, sems.at[0])
    out.start()
    out.wait()


@jax.jit
def pallas_sequential_preLN__compressed_kv_cla__moe_arch_mod__decode_kernel(
    A_x: jax.Array,
    A_c_kv: jax.Array,
    A_w_q: jax.Array,
    A_w_uk: jax.Array,
    A_w_uv: jax.Array,
    A_w_o: jax.Array,
    B_x: jax.Array,
    B_w_r: jax.Array,
    B_w_gate: jax.Array,
    B_w_up: jax.Array,
    B_w_down: jax.Array,
):
    del B_x
    hbm = pl.BlockSpec(memory_space=pl.ANY)
    return pl.pallas_call(
        _kernel,
        out_shape=jax.ShapeDtypeStruct((1, 1, M), A_x.dtype),
        in_specs=[hbm] * 10,
        out_specs=hbm,
        scratch_shapes=[
            pltpu.VMEM((1, 1, M), BF),
            pltpu.VMEM((M // LANES, LANES), BF),
            pltpu.VMEM((SK, DC), BF),
            pltpu.VMEM((M * H, D), BF),
            pltpu.VMEM((DC * H, D), BF),
            pltpu.VMEM((DC * H, D), BF),
            pltpu.VMEM((H * D, M), BF),
            pltpu.VMEM((F, M), BF),
            pltpu.VMEM((F, M), BF),
            pltpu.VMEM((F, M), BF),
            pltpu.VMEM((LANES, LANES), F32),
            pltpu.VMEM((SK // KB, H, KB), F32),
            pltpu.VMEM((H, D), F32),
            pltpu.VMEM((16, F), F32),
            pltpu.VMEM((16, M), F32),
            pltpu.VMEM((COL_TILES * LANES, LANES), F32),
            pltpu.VMEM((1, 1, M), BF),
            pltpu.SemaphoreType.DMA((NSEM,)),
        ],
        compiler_params=pltpu.CompilerParams(vmem_limit_bytes=64 * 2**20),
    )(A_x, A_c_kv.reshape(SK, DC), A_w_q.reshape(M * H, D), A_w_uk.reshape(DC * H, D),
      A_w_uv.reshape(DC * H, D), A_w_o.reshape(H * D, M), B_w_r.reshape(M // LANES, LANES),
      B_w_gate.T, B_w_up.T, B_w_down)
```

```python
import jax
import jax.numpy as jnp
from jax import lax
import jax.experimental.pallas as pl
import jax.experimental.pallas.tpu as pltpu

BF = jnp.bfloat16
F32 = jnp.float32
NT = (((1,), (1,)), ((), ()))
EPS = 1e-5

H, D, M, SK, DC, F = 32, 128, 512, 8192, 512, 1376
LANES = 128
TILES = 16
KB = 1024
OHEADS = 4
FCH = 256
NSEM = 3
DETOUR_O = (128, 128, 128, 160, 128)
DETOUR_DOWN = (64,)
DOWN_ROWS = (0, 640, 1024, 1264, 1344, F)
VPU_START = 1024
COL_TILES = -(-(F - VPU_START) // LANES)
COL_BASE = F - COL_TILES * LANES


def _layernorm(v):
    mean = jnp.mean(v, axis=-1, keepdims=True)
    d = v - mean
    var = jnp.mean(d * d, axis=-1, keepdims=True)
    return d / jnp.sqrt(var + EPS)


def _kernel(x_hbm, ckv_hbm, wq_hbm, wuk_hbm, wuv_hbm, wo_hbm, wr_hbm, wg_hbm, wu_hbm, wd_hbm,
            o_hbm,
            x_v, wr_v, ckv_v, wq_v, wuk_v, wuv_v, wo_v, wg_v, wu_v, wd_v,
            e_ref, s_ref, ctx_ref, hm_ref, y_ref, col_ref, o_v, stage, sems):
    down_chunks = list(zip(DOWN_ROWS[:-1], DOWN_ROWS[1:]))

    def rows(src, dst, a, b):
        return src.at[pl.ds(a, b - a)], dst.at[pl.ds(a, b - a)]

    groups = [
        [(wq_hbm, wq_v), (x_hbm, x_v), (wr_hbm, wr_v)],
        [(wuk_hbm, wuk_v)], [(ckv_hbm, ckv_v)], [(wuv_hbm, wuv_v)],
        [rows(wo_hbm, wo_v, sum(DETOUR_O), H * D)],
        [(wg_hbm, wg_v)], [(wu_hbm, wu_v)],
    ] + [[rows(wd_hbm, wd_v, max(a, sum(DETOUR_DOWN)), b)] for a, b in down_chunks]
    g_wq, g_wuk, g_ckv, g_wuv, g_wo, g_wg, g_wu, g_wd = range(8)
    copies = [[pltpu.make_async_copy(src, dst, sems.at[g % NSEM]) for src, dst in group]
              for g, group in enumerate(groups)]

    def start(g):
        if g < len(copies):
            for copy in copies[g]:
                copy.start()

    def wait(g):
        for copy in copies[g]:
            copy.wait()
        start(g + NSEM)

    detour = []
    for src, dst, sizes in ((wo_hbm, wo_v, DETOUR_O), (wd_hbm, wd_v, DETOUR_DOWN)):
        a = 0
        for n in sizes:
            piece = stage.at[pl.ds(0, n)]
            detour.append(pltpu.make_async_copy(src.at[pl.ds(a, n)], piece, sems.at[NSEM]))
            detour.append(pltpu.make_async_copy(piece, dst.at[pl.ds(a, n)], sems.at[NSEM]))
            a += n

    def advance_detour():
        detour.pop(0).wait()
        if detour:
            detour[0].start()

    detour[0].start()
    for g in range(NSEM):
        start(g)
    advance_detour()

    lane = lax.broadcasted_iota(jnp.int32, (H, LANES), 1)
    row = lax.broadcasted_iota(jnp.int32, (H, LANES), 0)
    own_head = (lane % H) == row

    def w_tile(w_ref, t):
        return jnp.concatenate(
            [w_ref[pl.ds(pl.multiple_of((i * LANES + t) * H, H), H), :] for i in range(4)], axis=0)

    def head_proj(w_ref, coef):
        e_ref[...] = coef.T

        def step(tb, acc):
            lhs, rhs = [], []
            for u in range(TILES):
                t = tb * TILES + u
                a = jnp.broadcast_to(e_ref[pl.ds(t, 1), :], (H, LANES))
                lhs.append(jnp.where(own_head, a, 0.0).astype(BF))
                rhs.append(w_tile(w_ref, t))
            return acc + jnp.dot(jnp.concatenate(lhs, axis=1), jnp.concatenate(rhs, axis=0),
                                 preferred_element_type=F32)

        return lax.fori_loop(0, LANES // TILES, step, jnp.zeros((H, D), F32))

    wait(g_wq)
    advance_detour()
    x = x_v[0].astype(F32)
    xn = _layernorm(x)
    q = head_proj(wq_v, jnp.concatenate(
        [jnp.broadcast_to(xn[:, i * LANES:(i + 1) * LANES], (H, LANES)) for i in range(4)], axis=0))
    q = q.astype(BF)

    advance_detour()
    wait(g_wuk)
    advance_detour()

    def absorb(tb, carry):
        rhs = jnp.concatenate([w_tile(wuk_v, tb * TILES + u) for u in range(TILES)], axis=0)
        r = lax.dot_general(q, rhs, NT, preferred_element_type=F32)
        for u in range(TILES):
            own = jnp.where(own_head, r[:, u * LANES:(u + 1) * LANES], 0.0)
            e_ref[pl.ds(tb * TILES + u, 1), :] = jnp.sum(own, axis=0, keepdims=True)
        return carry

    lax.fori_loop(0, LANES // TILES, absorb, 0)
    qa = e_ref[...].T * (D ** -0.5)
    qa = jnp.concatenate([qa[i * H:(i + 1) * H, :] for i in range(4)], axis=1).astype(BF)

    advance_detour()
    advance_detour()
    wait(g_ckv)
    advance_detour()

    def score(blk, mx):
        c = ckv_v[pl.ds(pl.multiple_of(blk * KB, KB), KB), :]
        s = lax.dot_general(qa, c, NT, preferred_element_type=F32)
        s_ref[blk] = s
        for u in range(KB // LANES):
            mx = jnp.maximum(mx, s[:, u * LANES:(u + 1) * LANES])
        return mx

    mx = lax.fori_loop(0, SK // KB, score, jnp.full((H, LANES), -jnp.inf, F32))
    advance_detour()
    row_max = jnp.max(mx, axis=1, keepdims=True)

    def attend(blk, carry):
        den, acc = carry
        p = jnp.exp(s_ref[blk] - row_max)
        for u in range(KB // LANES):
            den = den + p[:, u * LANES:(u + 1) * LANES]
        c = ckv_v[pl.ds(pl.multiple_of(blk * KB, KB), KB), :]
        return den, acc + jnp.dot(p.astype(BF), c, preferred_element_type=F32)

    den, acc = lax.fori_loop(0, SK // KB, attend,
                             (jnp.zeros((H, LANES), F32), jnp.zeros((H, DC), F32)))
    cc = acc / jnp.sum(den, axis=1, keepdims=True)

    coef = jnp.concatenate([cc[:, i * LANES:(i + 1) * LANES] for i in range(4)], axis=0)
    advance_detour()
    wait(g_wuv)
    ctx_ref[...] = head_proj(wuv_v, coef)

    advance_detour()
    assert len(detour) <= 2 * len(DETOUR_DOWN)
    wait(g_wo)

    def out_proj(hb, acc):
        lhs = jnp.concatenate(
            [jnp.broadcast_to(ctx_ref[pl.ds(hb * OHEADS + u, 1), :], (16, D)) for u in range(OHEADS)],
            axis=1)
        w = wo_v[pl.ds(pl.multiple_of(hb * (OHEADS * D), OHEADS * D), OHEADS * D), :]
        return acc + jnp.dot(lhs.astype(BF), w, preferred_element_type=F32)

    attn = lax.fori_loop(0, H // OHEADS, out_proj, jnp.zeros((16, M), F32))
    h = x + attn[0:1]
    hn = _layernorm(h)

    wr = wr_v[...].astype(F32)
    r = sum(jnp.sum(hn[:, i * LANES:(i + 1) * LANES] * wr[i:i + 1], axis=1, keepdims=True)
            for i in range(4))
    route = jax.nn.sigmoid(r)
    hn16 = jnp.broadcast_to(hn, (16, M)).astype(BF)
    f_chunks = [(a, min(a + FCH, F)) for a in range(0, F, FCH)]
    advance_detour()
    wait(g_wg)
    for a, b in f_chunks:
        g = lax.dot_general(hn16, wg_v[a:b, :], NT, preferred_element_type=F32)
        hm_ref[:, a:b] = g * jax.nn.sigmoid(g) * route
    wait(g_wu)
    for a, b in f_chunks:
        u = lax.dot_general(hn16, wu_v[a:b, :], NT, preferred_element_type=F32)
        hm_ref[:, a:b] = hm_ref[:, a:b] * u
    for t in range(COL_TILES):
        lo = COL_BASE + t * LANES
        col_ref[t * LANES:(t + 1) * LANES, :] = jnp.broadcast_to(
            hm_ref[0:1, lo:lo + LANES], (LANES, LANES)).T

    advance_detour()
    assert not detour
    y = jnp.broadcast_to(h + (hn + hn * 0.0), (16, M))
    y8 = None
    for j, (a, b) in enumerate(down_chunks):
        wait(g_wd + j)
        if a < VPU_START:
            y = y + jnp.dot(hm_ref[:, a:b].astype(BF), wd_v[a:b, :], preferred_element_type=F32)
            y_ref[...] = y
            continue
        if y8 is None:
            y8 = jnp.where(lax.broadcasted_iota(jnp.int32, (8, M), 0) == 0, y[0:8], 0.0)
        for r0 in range(a, b, 16):
            w = wd_v[r0:r0 + 16, :].astype(F32)
            unit = col_ref[r0 - COL_BASE:r0 - COL_BASE + 16, :]
            p = w * jnp.concatenate([unit] * (M // LANES), axis=1)
            y8 = y8 + (p[0:8] + p[8:16])
        if b < F:
            y_ref[0:8] = y8

    o_v[0] = jnp.sum(y8, axis=0, keepdims=True).astype(o_v.dtype)
    out = pltpu.make_async_copy(o_v, o_hbm, sems.at[0])
    out.start()
    out.wait()


@jax.jit
def pallas_sequential_preLN__compressed_kv_cla__moe_arch_mod__decode_kernel(
    A_x: jax.Array,
    A_c_kv: jax.Array,
    A_w_q: jax.Array,
    A_w_uk: jax.Array,
    A_w_uv: jax.Array,
    A_w_o: jax.Array,
    B_x: jax.Array,
    B_w_r: jax.Array,
    B_w_gate: jax.Array,
    B_w_up: jax.Array,
    B_w_down: jax.Array,
):
    del B_x
    hbm = pl.BlockSpec(memory_space=pl.ANY)
    return pl.pallas_call(
        _kernel,
        out_shape=jax.ShapeDtypeStruct((1, 1, M), A_x.dtype),
        in_specs=[hbm] * 10,
        out_specs=hbm,
        scratch_shapes=[
            pltpu.VMEM((1, 1, M), BF),
            pltpu.VMEM((M // LANES, LANES), BF),
            pltpu.VMEM((SK, DC), BF),
            pltpu.VMEM((M * H, D), BF),
            pltpu.VMEM((DC * H, D), BF),
            pltpu.VMEM((DC * H, D), BF),
            pltpu.VMEM((H * D, M), BF),
            pltpu.VMEM((F, M), BF),
            pltpu.VMEM((F, M), BF),
            pltpu.VMEM((F, M), BF),
            pltpu.VMEM((LANES, LANES), F32),
            pltpu.VMEM((SK // KB, H, KB), F32),
            pltpu.VMEM((H, D), F32),
            pltpu.VMEM((16, F), F32),
            pltpu.VMEM((16, M), F32),
            pltpu.VMEM((COL_TILES * LANES, LANES), F32),
            pltpu.VMEM((1, 1, M), BF),
            pltpu.SMEM((max(DETOUR_O + DETOUR_DOWN), M), BF),
            pltpu.SemaphoreType.DMA((NSEM + 1,)),
        ],
        compiler_params=pltpu.CompilerParams(vmem_limit_bytes=64 * 2**20),
    )(A_x, A_c_kv.reshape(SK, DC), A_w_q.reshape(M * H, D), A_w_uk.reshape(DC * H, D),
      A_w_uv.reshape(DC * H, D), A_w_o.reshape(H * D, M), B_w_r.reshape(M // LANES, LANES),
      B_w_gate.T, B_w_up.T, B_w_down)
```

```python
import jax
import jax.numpy as jnp
from jax import lax
import jax.experimental.pallas as pl
import jax.experimental.pallas.tpu as pltpu

BF = jnp.bfloat16
F32 = jnp.float32
NT = (((1,), (1,)), ((), ()))
EPS = 1e-5

H, D, M, SK, DC, F = 32, 128, 512, 8192, 512, 1376
LANES = 128
TILES = 16
KB = 1024
OHEADS = 4
FCH = 256
DETOUR = (("o", 128), ("o", 144), ("o", 112), ("o", 80), ("o", 96), ("g", 192), ("d", 80))
DOWN_ROWS = (0, 640, 1024, 1248, 1328, 1360, F)
VPU_START = 1024
COL_TILES = -(-(F - VPU_START) // LANES)
COL_BASE = F - COL_TILES * LANES


def _layernorm(v):
    mean = jnp.mean(v, axis=-1, keepdims=True)
    d = v - mean
    var = jnp.mean(d * d, axis=-1, keepdims=True)
    return d / jnp.sqrt(var + EPS)


def _body(x_hbm, ckv_hbm, wq_hbm, wuk_hbm, wuv_hbm, wo_hbm, wr_hbm, wg_hbm, wu_hbm, wd_hbm,
            o_hbm,
            x_v, wr_v, ckv_v, wq_v, wuk_v, wuv_v, wo_v, wg_v, wu_v, wd_v,
            e_ref, s_ref, ctx_ref, hm_ref, y_ref, col_ref, o_v, stage, sems, hop_sems):
    down_chunks = list(zip(DOWN_ROWS[:-1], DOWN_ROWS[1:]))

    def rows(src, dst, a, b):
        return src.at[pl.ds(a, b - a)], dst.at[pl.ds(a, b - a)]

    def staged(name):
        return sum(n for k, n in DETOUR if k == name)

    stream = [
        (wq_hbm, wq_v), (x_hbm, x_v), (wr_hbm, wr_v), (wuk_hbm, wuk_v), (ckv_hbm, ckv_v),
        (wuv_hbm, wuv_v), rows(wo_hbm, wo_v, staged("o"), H * D), rows(wg_hbm, wg_v, staged("g"), F),
        (wu_hbm, wu_v),
    ] + [rows(wd_hbm, wd_v, max(a, staged("d")), b) for a, b in down_chunks]
    stream = [pltpu.make_async_copy(src, dst, sems.at[i]) for i, (src, dst) in enumerate(stream)]
    c_wq, c_x, c_wr, c_wuk, c_ckv, c_wuv, c_wo, c_wg, c_wu, *c_wd = stream

    operands = {"o": (wo_hbm, wo_v), "g": (wg_hbm, wg_v), "d": (wd_hbm, wd_v)}
    to_smem, to_vmem, first_row, slot = [], [], dict.fromkeys(operands, 0), 0
    for i, (name, n) in enumerate(DETOUR):
        src, dst = rows(*operands[name], first_row[name], first_row[name] + n)
        piece = stage.at[pl.ds(slot, n)]
        to_smem.append(pltpu.make_async_copy(src, piece, hop_sems.at[2 * i]))
        to_vmem.append(pltpu.make_async_copy(piece, dst, hop_sems.at[2 * i + 1]))
        first_row[name] += n
        slot += n
    forwarded = []

    def advance_detour():
        i = len(forwarded)
        to_smem[i].wait()
        to_vmem[i].start()
        if i + 1 < len(DETOUR):
            to_smem[i + 1].start()
        forwarded.append(i)

    def land(name):
        for i, (k, _) in enumerate(DETOUR):
            if k == name:
                assert i in forwarded
                to_vmem[i].wait()

    to_smem[0].start()
    for copy in stream:
        copy.start()
    advance_detour()

    lane = lax.broadcasted_iota(jnp.int32, (H, LANES), 1)
    row = lax.broadcasted_iota(jnp.int32, (H, LANES), 0)
    own_head = (lane % H) == row

    def w_tile(w_ref, t):
        return jnp.concatenate(
            [w_ref[pl.ds(pl.multiple_of((i * LANES + t) * H, H), H), :] for i in range(4)], axis=0)

    def head_proj(w_ref, coef):
        e_ref[...] = coef.T

        def step(tb, acc):
            lhs, rhs = [], []
            for u in range(TILES):
                t = tb * TILES + u
                a = jnp.broadcast_to(e_ref[pl.ds(t, 1), :], (H, LANES))
                lhs.append(jnp.where(own_head, a, 0.0).astype(BF))
                rhs.append(w_tile(w_ref, t))
            return acc + jnp.dot(jnp.concatenate(lhs, axis=1), jnp.concatenate(rhs, axis=0),
                                 preferred_element_type=F32)

        return lax.fori_loop(0, LANES // TILES, step, jnp.zeros((H, D), F32))

    c_wq.wait()
    c_x.wait()
    x = x_v[0].astype(F32)
    xn = _layernorm(x)
    q = head_proj(wq_v, jnp.concatenate(
        [jnp.broadcast_to(xn[:, i * LANES:(i + 1) * LANES], (H, LANES)) for i in range(4)], axis=0))
    q = q.astype(BF)

    advance_detour()
    c_wuk.wait()

    def absorb(tb, carry):
        rhs = jnp.concatenate([w_tile(wuk_v, tb * TILES + u) for u in range(TILES)], axis=0)
        r = lax.dot_general(q, rhs, NT, preferred_element_type=F32)
        for u in range(TILES):
            own = jnp.where(own_head, r[:, u * LANES:(u + 1) * LANES], 0.0)
            e_ref[pl.ds(tb * TILES + u, 1), :] = jnp.sum(own, axis=0, keepdims=True)
        return carry

    lax.fori_loop(0, LANES // TILES, absorb, 0)
    qa = e_ref[...].T * (D ** -0.5)
    qa = jnp.concatenate([qa[i * H:(i + 1) * H, :] for i in range(4)], axis=1).astype(BF)

    advance_detour()
    advance_detour()
    c_ckv.wait()
    advance_detour()

    def score(blk, mx):
        c = ckv_v[pl.ds(pl.multiple_of(blk * KB, KB), KB), :]
        s = lax.dot_general(qa, c, NT, preferred_element_type=F32)
        s_ref[blk] = s
        for u in range(KB // LANES):
            mx = jnp.maximum(mx, s[:, u * LANES:(u + 1) * LANES])
        return mx

    mx = lax.fori_loop(0, SK // KB, score, jnp.full((H, LANES), -jnp.inf, F32))
    row_max = jnp.max(mx, axis=1, keepdims=True)

    def attend(blk, carry):
        den, acc = carry
        p = jnp.exp(s_ref[blk] - row_max)
        for u in range(KB // LANES):
            den = den + p[:, u * LANES:(u + 1) * LANES]
        c = ckv_v[pl.ds(pl.multiple_of(blk * KB, KB), KB), :]
        return den, acc + jnp.dot(p.astype(BF), c, preferred_element_type=F32)

    den, acc = lax.fori_loop(0, SK // KB, attend,
                             (jnp.zeros((H, LANES), F32), jnp.zeros((H, DC), F32)))
    cc = acc / jnp.sum(den, axis=1, keepdims=True)

    coef = jnp.concatenate([cc[:, i * LANES:(i + 1) * LANES] for i in range(4)], axis=0)
    advance_detour()
    c_wuv.wait()
    ctx_ref[...] = head_proj(wuv_v, coef)

    c_wo.wait()
    land("o")

    def out_proj(hb, acc):
        lhs = jnp.concatenate(
            [jnp.broadcast_to(ctx_ref[pl.ds(hb * OHEADS + u, 1), :], (16, D)) for u in range(OHEADS)],
            axis=1)
        w = wo_v[pl.ds(pl.multiple_of(hb * (OHEADS * D), OHEADS * D), OHEADS * D), :]
        return acc + jnp.dot(lhs.astype(BF), w, preferred_element_type=F32)

    attn = lax.fori_loop(0, H // OHEADS, out_proj, jnp.zeros((16, M), F32))
    h = x + attn[0:1]
    hn = _layernorm(h)

    c_wr.wait()
    wr = wr_v[...].astype(F32)
    r = sum(jnp.sum(hn[:, i * LANES:(i + 1) * LANES] * wr[i:i + 1], axis=1, keepdims=True)
            for i in range(4))
    route = jax.nn.sigmoid(r)
    hn16 = jnp.broadcast_to(hn, (16, M)).astype(BF)
    f_chunks = [(a, min(a + FCH, F)) for a in range(0, F, FCH)]
    advance_detour()
    c_wg.wait()
    land("g")
    for a, b in f_chunks:
        g = lax.dot_general(hn16, wg_v[a:b, :], NT, preferred_element_type=F32)
        hm_ref[:, a:b] = g * jax.nn.sigmoid(g) * route
    c_wu.wait()
    for a, b in f_chunks:
        u = lax.dot_general(hn16, wu_v[a:b, :], NT, preferred_element_type=F32)
        hm_ref[:, a:b] = hm_ref[:, a:b] * u
    for t in range(COL_TILES):
        lo = COL_BASE + t * LANES
        col_ref[t * LANES:(t + 1) * LANES, :] = jnp.broadcast_to(
            hm_ref[0:1, lo:lo + LANES], (LANES, LANES)).T

    land("d")
    y = jnp.broadcast_to(h + (hn + hn * 0.0), (16, M))
    y8 = None
    for j, (a, b) in enumerate(down_chunks):
        c_wd[j].wait()
        if a < VPU_START:
            y = y + jnp.dot(hm_ref[:, a:b].astype(BF), wd_v[a:b, :], preferred_element_type=F32)
            y_ref[...] = y
            continue
        if y8 is None:
            y8 = jnp.where(lax.broadcasted_iota(jnp.int32, (8, M), 0) == 0, y[0:8], 0.0)
        for r0 in range(a, b, 16):
            w = wd_v[r0:r0 + 16, :].astype(F32)
            unit = col_ref[r0 - COL_BASE:r0 - COL_BASE + 16, :]
            p = w * jnp.concatenate([unit] * (M // LANES), axis=1)
            y8 = y8 + (p[0:8] + p[8:16])
        if b < F:
            y_ref[0:8] = y8

    o_v[0] = jnp.sum(y8, axis=0, keepdims=True).astype(o_v.dtype)
    out = pltpu.make_async_copy(o_v, o_hbm, sems.at[0])
    out.start()
    out.wait()


def _kernel(*refs):
    pl.run_scoped(lambda *sems: _body(*refs, *sems),
                  pltpu.SemaphoreType.DMA((9 + len(DOWN_ROWS) - 1,)),
                  pltpu.SemaphoreType.DMA((2 * len(DETOUR),)))


@jax.jit
def pallas_sequential_preLN__compressed_kv_cla__moe_arch_mod__decode_kernel(
    A_x: jax.Array,
    A_c_kv: jax.Array,
    A_w_q: jax.Array,
    A_w_uk: jax.Array,
    A_w_uv: jax.Array,
    A_w_o: jax.Array,
    B_x: jax.Array,
    B_w_r: jax.Array,
    B_w_gate: jax.Array,
    B_w_up: jax.Array,
    B_w_down: jax.Array,
):
    del B_x
    hbm = pl.BlockSpec(memory_space=pl.ANY)
    return pl.pallas_call(
        _kernel,
        out_shape=jax.ShapeDtypeStruct((1, 1, M), A_x.dtype),
        in_specs=[hbm] * 10,
        out_specs=hbm,
        scratch_shapes=[
            pltpu.VMEM((1, 1, M), BF),
            pltpu.VMEM((M // LANES, LANES), BF),
            pltpu.VMEM((SK, DC), BF),
            pltpu.VMEM((M * H, D), BF),
            pltpu.VMEM((DC * H, D), BF),
            pltpu.VMEM((DC * H, D), BF),
            pltpu.VMEM((H * D, M), BF),
            pltpu.VMEM((F, M), BF),
            pltpu.VMEM((F, M), BF),
            pltpu.VMEM((F, M), BF),
            pltpu.VMEM((LANES, LANES), F32),
            pltpu.VMEM((SK // KB, H, KB), F32),
            pltpu.VMEM((H, D), F32),
            pltpu.VMEM((16, F), F32),
            pltpu.VMEM((16, M), F32),
            pltpu.VMEM((COL_TILES * LANES, LANES), F32),
            pltpu.VMEM((1, 1, M), BF),
            pltpu.SMEM((sum(n for _, n in DETOUR), M), BF),
        ],
        compiler_params=pltpu.CompilerParams(vmem_limit_bytes=64 * 2**20),
    )(A_x, A_c_kv.reshape(SK, DC), A_w_q.reshape(M * H, D), A_w_uk.reshape(DC * H, D),
      A_w_uv.reshape(DC * H, D), A_w_o.reshape(H * D, M), B_w_r.reshape(M // LANES, LANES),
      B_w_gate.T, B_w_up.T, B_w_down)
```
